```python
import jax
import jax.numpy as jnp

def _softmax(x, axis=-1):
    return jax.nn.softmax(x, axis=axis)
def _gelu(x):
    return jax.nn.gelu(x, approximate=True)
def _silu(x):
    return jax.nn.silu(x)
def _sigmoid(x):
    return jax.nn.sigmoid(x)
def _layernorm(x, axis=-1, eps=1e-5):
    m = jnp.mean(x, axis=axis, keepdims=True)
    v = jnp.var(x, axis=axis, keepdims=True)
    return (x - m) / jnp.sqrt(v + eps)
def _scatter_add(tgt, idx, src, axis=0):
    return tgt.at[idx].add(src)
def _segment_sum(src, seg, n):
    return jax.ops.segment_sum(src, seg, n)
class _Rng:
    def __init__(self, key):
        self._k = key
    def _next(self):
        self._k, sub = jax.random.split(self._k)
        return sub
    def normal(self, shape):
        return jax.random.normal(self._next(), shape, dtype=jnp.bfloat16)
    def randint(self, lo, hi, shape):
        return jax.random.randint(self._next(), shape, lo, hi, dtype=jnp.int32)
    def uniform(self, shape, lo=0.0, hi=1.0):
        return jax.random.uniform(self._next(), shape, jnp.bfloat16, lo, hi)
    def permutation(self, n):
        return jax.random.permutation(self._next(), n)


kernel_name = 'interleave_layers__sliding_block__moe_arch_mod__prompt'

def setup_inputs():
    _rng = _Rng(jax.random.key(int.from_bytes(__import__("os").urandom(4), "little")))
    _w = (lambda a: (lambda t: t.astype(jnp.bfloat16) if jnp.issubdtype(t.dtype, jnp.floating) else t)(jnp.asarray(a)))
    def _A_setup():
        B, S, D = 1, 2048, 1024
        return {
            "x": _w((lambda *s: _rng.normal(s) * 0.05)(B, S, D)),
            "wqkv": _w((lambda *s: _rng.normal(s) * 0.05)(D, 3 * D)),
            "wo": _w((lambda *s: _rng.normal(s) * 0.05)(D, D)),
        }
    _A_in = _A_setup()

    def _B_setup():
        B, S, D, F, C = 1, 2048, 1024, 3584, 1
        return {
            "x": _w((lambda *s: _rng.normal(s) * 0.05)(B, S, D)),
            "w_r": _w((lambda *s: _rng.normal(s) * 0.05)(D)),
            "w_gate": _w((lambda *s: _rng.normal(s) * 0.05)(D, F)),
            "w_up": _w((lambda *s: _rng.normal(s) * 0.05)(D, F)),
            "w_down": _w((lambda *s: _rng.normal(s) * 0.05)(F, D)),
        }
    _B_in = _B_setup()

    return {
        "A_x": _A_in["x"],
        "A_wqkv": _A_in["wqkv"],
        "A_wo": _A_in["wo"],
        "B_x": _B_in["x"],
        "B_w_r": _B_in["w_r"],
        "B_w_gate": _B_in["w_gate"],
        "B_w_up": _B_in["w_up"],
        "B_w_down": _B_in["w_down"],
    }

def reference(A_x, A_wqkv, A_wo, B_x, B_w_r, B_w_gate, B_w_up, B_w_down):
    def _A_ref(x, wqkv, wo):
        B, S, D = x.shape
        H = 32; Dh = D // H; W = 256
        qkv = (lambda x, *d: x.transpose(*d))((x @ wqkv).reshape(B, S, 3, H, Dh), 2, 0, 3, 1, 4)
        q, k, v = qkv[0], qkv[1], qkv[2]
        scores = jnp.einsum("bhqd,bhkd->bhqk", q, k) * (Dh ** -0.5)
        idx = jnp.arange(S)
        mask = (idx[:, None] - idx[None, :] >= 0) & (idx[:, None] - idx[None, :] < W)
        scores = jnp.where(mask[None, None], scores, -1e9)
        p = _softmax(scores, axis=-1)
        o = jnp.einsum("bhqk,bhkd->bhqd", p, v)
        return (lambda x, *d: x.transpose(*d))(o, 0, 2, 1, 3).reshape(B, S, D) @ wo

    def _B_ref(x, w_r, w_gate, w_up, w_down):
        B, S, D = x.shape
        C = 1
        r = x @ w_r
        idx = jnp.argsort(-r, axis=-1)[:, :C]
        idx_e = jnp.repeat(idx.reshape(B, C, 1), D, axis=2)
        x_sel = jnp.take_along_axis(x, idx_e, axis=1)
        g = _silu(x_sel @ w_gate)
        u = x_sel @ w_up
        y = (g * u) @ w_down
        r_sel = _sigmoid(jnp.take_along_axis(r, idx, axis=1))
        y = y * r_sel.reshape(B, C, 1)
        b_off = (jnp.arange(B) * S).reshape(B, 1)
        flat_idx = (idx + b_off).reshape(B * C)
        zero = (x * 0.0).reshape(B * S, D)
        upd = _scatter_add(zero, flat_idx, y.reshape(B * C, D), axis=0)
        return x + upd.reshape(B, S, D)

    x = A_x
    x = x + _A_ref(_layernorm(x, axis=-1), A_wqkv, A_wo)
    x = x + _B_ref(_layernorm(x, axis=-1), B_w_r, B_w_gate, B_w_up, B_w_down)
    x = x + _A_ref(_layernorm(x, axis=-1), A_wqkv, A_wo)
    x = x + _B_ref(_layernorm(x, axis=-1), B_w_r, B_w_gate, B_w_up, B_w_down)
    return x
```

```python
import jax
import jax.numpy as jnp
from jax import lax
import jax.experimental.pallas as pl
import jax.experimental.pallas.tpu as pltpu

S = 2048
D = 1024
F = 3584
DH = 32
NG = D // 128
NT = S // 128
RC = 512
EPS = 1e-5
NEG = -1e9
LOG2E = 1.4426950408889634
SCALE = 0.1767578125
WO_CHUNKS = (256, 256, 256, 256, 256, 256, 256, 128, 128)

bf16 = jnp.bfloat16
f32 = jnp.float32
u32 = jnp.uint32


def _round_bf16(v):
    return v.astype(bf16).astype(f32)


def _layernorm(x):
    m = jnp.sum(x, axis=-1, keepdims=True) * (1.0 / D)
    c = x - m
    v = jnp.sum(c * c, axis=-1, keepdims=True) * (1.0 / D)
    s = _round_bf16(jnp.sqrt(_round_bf16(_round_bf16(v) + EPS)))
    return (x - _round_bf16(m)) * (1.0 / s)


def _kernel(x_hbm, wqkv_hbm, wo_hbm, wr_ref, wg_hbm, wu_hbm, wd_hbm, out_hbm,
            x_ref, xn_ref, q_ref, k_ref, vt_ref, o_ref,
            wqkv_ref, wo_ref, wg_ref, wu_ref, wd_ref,
            s_ref, m_ref, in_sem, out_sem):
    nrc = S // RC

    def x_copy(c):
        rows = pl.ds(c * RC, RC)
        return pltpu.make_async_copy(x_hbm.at[0, rows], x_ref.at[rows], in_sem.at[c])

    wq_copy = pltpu.make_async_copy(
        wqkv_hbm.at[:, 0:D], wqkv_ref.at[:, 0:D], in_sem.at[nrc])
    wkv_copy = pltpu.make_async_copy(
        wqkv_hbm.at[:, D:3 * D], wqkv_ref.at[:, D:3 * D], in_sem.at[nrc + 1])
    wo_copy = pltpu.make_async_copy(wo_hbm, wo_ref, in_sem.at[nrc + 2])
    wg_copy = pltpu.make_async_copy(wg_hbm, wg_ref, in_sem.at[nrc + 3])
    wu_copy = pltpu.make_async_copy(wu_hbm, wu_ref, in_sem.at[nrc + 4])
    wd_copy = pltpu.make_async_copy(wd_hbm, wd_ref, in_sem.at[nrc + 5])

    def out_copy(i, r0, n):
        rows = pl.ds(r0, n)
        return pltpu.make_async_copy(x_ref.at[rows], out_hbm.at[0, rows], out_sem.at[i])

    def ln_chunk(c):
        rows = pl.ds(pl.multiple_of(c * RC, RC), RC)
        xn_ref[rows, :] = _layernorm(x_ref[rows, :].astype(f32)).astype(bf16)

    def store_groups(dst, c, val):
        half = pl.ds(pl.multiple_of(c * (RC // 2), RC // 2), RC // 2)
        for g in range(NG):
            dst[g, half, :] = pltpu.bitcast(
                val[:, g * 128:(g + 1) * 128].astype(bf16), u32)

    def tri():
        return (lax.broadcasted_iota(jnp.int32, (16, 128), 0)
                - lax.broadcasted_iota(jnp.int32, (16, 128), 1))

    def scores(g, t):
        slot = t % 2
        parts = []
        for j in range(8):
            if t >= 2:
                parts.append(k_ref[g, (t - 2) * 64 + j * 8:(t - 2) * 64 + j * 8 + 8, :])
            parts.append(k_ref[g, t * 64 + j * 8:t * 64 + j * 8 + 8, :])
        if t >= 1:
            parts.append(k_ref[g, (t - 1) * 64:t * 64, :])
        kw = pltpu.bitcast(jnp.concatenate(parts, axis=0), bf16)
        qt = q_ref[g, t * 64:(t + 1) * 64, :]
        head = lax.broadcasted_iota(jnp.int32, (64, 128), 1) >> 5
        w = jnp.concatenate(
            [jnp.where(head == h, qt, jnp.zeros_like(qt)) for h in range(4)], axis=0)
        s = lax.dot_general(kw, pltpu.bitcast(w, bf16), (((1,), (1,)), ((), ())),
                            preferred_element_type=f32)
        d = tri()
        ms = [None] * 4
        for j in range(8):
            old = d > -16 * j
            for h in range(4):
                cols = slice(h * 128, (h + 1) * 128)
                if t >= 2:
                    sm = jnp.where(old, s[32 * j:32 * j + 16, cols],
                                   s[32 * j + 16:32 * j + 32, cols])
                else:
                    sm = jnp.where(old, NEG, s[16 * j:16 * j + 16, cols])
                s_ref[slot, h, 16 * j:16 * j + 16, :] = sm
                mm = jnp.maximum(sm[0:8], sm[8:16])
                ms[h] = mm if ms[h] is None else jnp.maximum(ms[h], mm)
        if t >= 1:
            base = 256 if t >= 2 else 128
            for j in range(8):
                for h in range(4):
                    sm = s[base + 16 * j:base + 16 * j + 16, h * 128:(h + 1) * 128]
                    s_ref[slot, h, 128 + 16 * j:128 + 16 * j + 16, :] = sm
                    ms[h] = jnp.maximum(ms[h], jnp.maximum(sm[0:8], sm[8:16]))
        for h in range(4):
            m_ref[slot, h] = jnp.broadcast_to(
                jnp.max(ms[h], axis=0, keepdims=True), (8, 128))

    def attend(g, t):
        slot = t % 2
        d = tri()
        outs = []
        for h in range(4):
            m = m_ref[slot, h]
            m2 = jnp.concatenate([m, m], axis=0)
            l = None
            p_old, p_mid, p_new = [None] * 8, [None] * 8, [None] * 8
            for j in reversed(range(16 if t >= 1 else 8)):
                p = jnp.exp2(s_ref[slot, h, 16 * j:16 * j + 16, :] - m2)
                pp = p[0:8] + p[8:16]
                l = pp if l is None else l + pp
                if j >= 8:
                    p_mid[j - 8] = p
                elif t >= 2:
                    old = d > -16 * j
                    p_old[j] = jnp.where(old, p, 0.0)
                    p_new[j] = jnp.where(old, 0.0, p)
                else:
                    p_new[j] = jnp.where(d > -16 * j, 0.0, p)
            ps = (p_old if t >= 2 else []) + (p_mid if t >= 1 else []) + p_new
            p = jnp.concatenate(ps, axis=0).astype(bf16)
            rows = pl.ds(pl.multiple_of(g * 64 + h * 16, 16), 16)
            vt = jnp.concatenate(
                [vt_ref[b, rows, :] for b in range(max(t - 2, 0), t + 1)], axis=1)
            o = jnp.dot(pltpu.bitcast(vt, bf16), p, preferred_element_type=f32)
            outs.append(o * (1.0 / jnp.sum(l, axis=0, keepdims=True)))
        ot = jnp.concatenate(outs, axis=0)
        o_ref[g, t * 128:(t + 1) * 128, :] = ot.T.astype(bf16)

    def layer(li, carry):
        first = li == 0

        @pl.when(first)
        def _():
            x_copy(0).start()
            wq_copy.start()
            x_copy(0).wait()
            for c in range(1, nrc):
                x_copy(c).start()
            wkv_copy.start()

        ln_chunk(0)

        @pl.when(first)
        def _():
            wq_copy.wait()

        def q_body(c, _):
            nxt = jnp.minimum(c + 1, nrc - 1)

            @pl.when(jnp.logical_and(first, c + 1 < nrc))
            def _():
                x_copy(nxt).wait()

            rows = pl.ds(pl.multiple_of(c * RC, RC), RC)
            q = jnp.dot(xn_ref[rows, :], wqkv_ref[:, 0:D], preferred_element_type=f32)
            store_groups(q_ref, c, q * (SCALE * LOG2E))
            ln_chunk(nxt)
            return _

        lax.fori_loop(0, nrc, q_body, None)

        @pl.when(first)
        def _():
            wo_copy.start()
            wg_copy.start()
            wu_copy.start()
            wd_copy.start()
            wkv_copy.wait()

        def kv_body(c, _):
            rows = pl.ds(pl.multiple_of(c * RC, RC), RC)
            xn = xn_ref[rows, :]
            v = jnp.dot(xn, wqkv_ref[:, 2 * D:3 * D], preferred_element_type=f32)
            for g in range(NG):
                for b in range(RC // 128):
                    vt = v[b * 128:(b + 1) * 128, g * 128:(g + 1) * 128].T
                    vt_ref[c * (RC // 128) + b, g * 64:(g + 1) * 64, :] = pltpu.bitcast(
                        vt.astype(bf16), u32)
            k = jnp.dot(xn, wqkv_ref[:, D:2 * D], preferred_element_type=f32)
            store_groups(k_ref, c, k)
            return _

        lax.fori_loop(0, nrc, kv_body, None)

        def att_body(g, _):
            scores(g, 0)
            for t in range(NT):
                if t + 1 < NT:
                    scores(g, t + 1)
                attend(g, t)
            return _

        lax.fori_loop(0, NG, att_body, None)

        @pl.when(first)
        def _():
            wo_copy.wait()
            wg_copy.wait()
            wu_copy.wait()
            wd_copy.wait()

        wr = wr_ref[...].astype(f32).reshape(1, D)
        best = jnp.full((8, 1), -jnp.inf, f32)
        best_i = jnp.zeros((8, 1), jnp.int32)
        sub = lax.broadcasted_iota(jnp.int32, (8, 1), 0)
        r0 = 0
        for i, n in enumerate(WO_CHUNKS):
            o = jnp.concatenate([o_ref[g, r0:r0 + n, :] for g in range(NG)], axis=1)
            a = jnp.dot(o, wo_ref[...], preferred_element_type=f32)
            x1 = x_ref[r0:r0 + n, :].astype(f32) + a
            ln = _layernorm(x1)
            r = jnp.sum(ln * wr, axis=-1, keepdims=True)
            xn_ref[r0:r0 + n, :] = ln.astype(bf16)
            x_ref[r0:r0 + n, :] = (x1 + ln).astype(bf16)
            out_copy(i, r0, n).start()
            for j in range(n // 8):
                rj = r[8 * j:8 * j + 8]
                take = rj > best
                best = jnp.where(take, rj, best)
                best_i = jnp.where(take, sub + (r0 + 8 * j), best_i)
            r0 += n

        top = jnp.max(best, axis=0, keepdims=True)
        idx = jnp.min(jnp.where(best == top, best_i, S - 1))
        base = pl.multiple_of((idx >> 4) << 4, 16)
        tile = pl.ds(base, 16)
        xs = xn_ref[tile, :]
        gate = jnp.dot(xs, wg_ref[...], preferred_element_type=f32)
        up = jnp.dot(xs, wu_ref[...], preferred_element_type=f32)
        hid = (gate * jax.nn.sigmoid(gate) * up).astype(bf16)
        y = jnp.dot(hid, wd_ref[...], preferred_element_type=f32) * jax.nn.sigmoid(top)
        xt = x_ref[tile, :].astype(f32)
        hit = lax.broadcasted_iota(jnp.int32, (16, D), 0) == idx - base
        new = jnp.where(hit, xt + y, xt).astype(bf16)
        r0 = 0
        for i, n in enumerate(WO_CHUNKS):
            out_copy(i, r0, n).wait()
            r0 += n
        x_ref[tile, :] = new

        @pl.when(jnp.logical_not(first))
        def _():
            fix = out_copy(0, base, 16)
            fix.start()
            fix.wait()

        return carry

    lax.fori_loop(0, 2, layer, None)


@jax.jit
def pallas_interleave_layers__sliding_block__moe_arch_mod__prompt_kernel(
    A_x: jax.Array,
    A_wqkv: jax.Array,
    A_wo: jax.Array,
    B_x: jax.Array,
    B_w_r: jax.Array,
    B_w_gate: jax.Array,
    B_w_up: jax.Array,
    B_w_down: jax.Array,
):
    del B_x
    hbm = pl.BlockSpec(memory_space=pl.ANY)
    return pl.pallas_call(
        _kernel,
        out_shape=jax.ShapeDtypeStruct((1, S, D), bf16),
        in_specs=[hbm, hbm, hbm, pl.BlockSpec(memory_space=pltpu.VMEM), hbm, hbm, hbm],
        out_specs=hbm,
        scratch_shapes=[
            pltpu.VMEM((S, D), bf16),
            pltpu.VMEM((S, D), bf16),
            pltpu.VMEM((NG, S // 2, 128), u32),
            pltpu.VMEM((NG, S // 2, 128), u32),
            pltpu.VMEM((NT, D // 2, 128), u32),
            pltpu.VMEM((NG, S, 128), bf16),
            pltpu.VMEM((D, 3 * D), bf16),
            pltpu.VMEM((D, D), bf16),
            pltpu.VMEM((D, F), bf16),
            pltpu.VMEM((D, F), bf16),
            pltpu.VMEM((F, D), bf16),
            pltpu.VMEM((2, 4, 256, 128), f32),
            pltpu.VMEM((2, 4, 8, 128), f32),
            pltpu.SemaphoreType.DMA((S // RC + 6,)),
            pltpu.SemaphoreType.DMA((len(WO_CHUNKS),)),
        ],
        compiler_params=pltpu.CompilerParams(vmem_limit_bytes=100 * 2**20),
    )(A_x, A_wqkv, A_wo, B_w_r, B_w_gate, B_w_up, B_w_down)
```

```python
import jax
import jax.numpy as jnp
from jax import lax
import jax.experimental.pallas as pl
import jax.experimental.pallas.tpu as pltpu

S = 2048
D = 1024
F = 3584
DH = 32
NG = D // 128
NT = S // 128
RC = 512
EPS = 1e-5
NEG = -1e9
LOG2E = 1.4426950408889634
SCALE = 0.1767578125
X_EDGES = (0, 640, 1152, 1664, 2048)
OUT_ROWS = 256

bf16 = jnp.bfloat16
f32 = jnp.float32
u32 = jnp.uint32


def _round_bf16(v):
    return v.astype(bf16).astype(f32)


def _layernorm(x):
    m = jnp.sum(x, axis=-1, keepdims=True) * (1.0 / D)
    c = x - m
    v = jnp.sum(c * c, axis=-1, keepdims=True) * (1.0 / D)
    s = _round_bf16(jnp.sqrt(_round_bf16(_round_bf16(v) + EPS)))
    return (x - _round_bf16(m)) * (1.0 / s)


def _token(vals, zero):
    acc = None
    for v in vals:
        b = pltpu.bitcast(v, u32)
        for i in range(b.shape[0] // 8):
            for j in range(b.shape[1] // 128):
                t = b[8 * i:8 * i + 8, 128 * j:128 * j + 128]
                acc = t if acc is None else acc | t
    return acc & zero


def _after(w, token):
    if token is None:
        return w
    b = pltpu.bitcast(w, u32)
    return pltpu.bitcast(jnp.concatenate([b[0:8] | token, b[8:]], axis=0), bf16)


def _regroup(xs, lane):
    def sel(c, a, b):
        if a is None and b is None:
            return None
        return jnp.where(c, 0.0 if a is None else a, 0.0 if b is None else b)

    for bit in (1, 2):
        c = (lane & (32 * bit)) != 0
        xs = [sel(c, xs[h ^ bit], xs[h]) for h in range(4)]
    return xs


def _kernel(x_hbm, wqkv_hbm, wo_hbm, wr_ref, wg_hbm, wu_hbm, wd_hbm, out_hbm,
            x_ref, xn_ref, q_ref, k_ref, vt_ref, o_ref,
            wqkv_ref, wo_ref, wg_ref, wu_ref, wd_ref,
            s_ref, m_ref, cur_ref, a_ref, x_sem, w_sem, out_sem):
    nrc = S // RC

    def x_copy(c):
        rows = pl.ds(X_EDGES[c], X_EDGES[c + 1] - X_EDGES[c])
        return pltpu.make_async_copy(x_hbm.at[0, rows], x_ref.at[rows], x_sem.at[c])

    def wqkv_copy(part, lo, hi, sem):
        cols = pl.ds(part * D + lo, hi - lo)
        return pltpu.make_async_copy(
            wqkv_hbm.at[:, cols], wqkv_ref.at[:, cols], w_sem.at[sem])

    head_copies = [wqkv_copy(i, 0, 128, i) for i in range(3)]
    rest_copies = [wqkv_copy(i, 128, D, 3 + i) for i in range(3)]
    late_copies = [
        pltpu.make_async_copy(src, dst, w_sem.at[6 + i])
        for i, (src, dst) in enumerate(
            [(wo_hbm, wo_ref), (wg_hbm, wg_ref), (wu_hbm, wu_ref), (wd_hbm, wd_ref)])]

    def out_copy(i, r0, n):
        rows = pl.ds(r0, n)
        return pltpu.make_async_copy(x_ref.at[rows], out_hbm.at[0, rows], out_sem.at[i])

    def ln_piece(blk, j, slot):
        rows = pl.ds(pl.multiple_of(blk * 128 + j * 16, 16), 16)
        ln = _layernorm(x_ref[rows, :].astype(f32))
        xn = ln.astype(bf16)
        xn_ref[rows, :] = xn
        cur_ref[slot, j * 16:(j + 1) * 16, :] = xn
        return ln

    def project(part, g, blk, xn, token=None):
        cols = pl.ds(pl.multiple_of(part * D + g * 128, 128), 128)
        y = jnp.dot(xn, _after(wqkv_ref[:, cols], token), preferred_element_type=f32)
        if part == 0:
            y = y * (SCALE * LOG2E)
        if part == 2:
            y = y.T
        (q_ref, k_ref, vt_ref)[part][blk] = pltpu.bitcast(y.astype(bf16), u32)

    def tri():
        return (lax.broadcasted_iota(jnp.int32, (16, 128), 0)
                - (lax.broadcasted_iota(jnp.int32, (16, 128), 1) & 31))

    def scores(t):
        slot = t % 2
        head = lax.broadcasted_iota(jnp.int32, (16, 128), 1) >> 5
        tiles = []
        for j in range(4):
            k0 = t * 128 + j * 32 - 256
            order = [c for c in [0, 16, 1, 17] + list(range(2, 16)) if k0 + 16 * c >= 0]
            parts = []
            for c in order:
                key = k0 + 16 * c
                parts.append(k_ref[key // 128, key % 128 // 2:key % 128 // 2 + 8, :])
            kw = pltpu.bitcast(jnp.concatenate(parts, axis=0), bf16)
            qt = q_ref[t, j * 16:(j + 1) * 16, :]
            w = jnp.concatenate(
                [jnp.where(head == (s ^ j), qt, jnp.zeros_like(qt)) for s in range(4)],
                axis=0)
            sc = lax.dot_general(kw, pltpu.bitcast(w, bf16), (((1,), (1,)), ((), ())),
                                 preferred_element_type=f32)
            tiles.append({c: sc[16 * i:16 * i + 16] for i, c in enumerate(order)})
        d = tri()
        ms = [None] * 4
        for c in range(16):
            for j in range(4):
                if c < 2:
                    sm = jnp.where(d > -16 * c, tiles[j].get(c, NEG), tiles[j][c + 16])
                elif c in tiles[j]:
                    sm = tiles[j][c]
                else:
                    continue
                s_ref[slot, j, 16 * c:16 * c + 16, :] = sm
                mm = jnp.maximum(sm[0:8], sm[8:16])
                ms[j] = mm if ms[j] is None else jnp.maximum(ms[j], mm)
        for j in range(4):
            m_ref[slot, j] = jnp.broadcast_to(
                jnp.max(ms[j], axis=0, keepdims=True), (8, 128))

    def attend(g, t):
        slot = t % 2
        d = tri()
        lane = lax.broadcasted_iota(jnp.int32, (16, 128), 1)
        m2 = [jnp.concatenate([m_ref[slot, j]] * 2, axis=0) for j in range(4)]
        l = [None] * 4
        probs = {}

        def prob(j, key):
            c = (key - (t * 128 + j * 32 - 256)) // 16
            if c < 0 or c >= 18:
                return None
            cm = c % 16
            if (j, cm) not in probs:
                p = jnp.exp2(s_ref[slot, j, 16 * cm:16 * cm + 16, :] - m2[j])
                pp = p[0:8] + p[8:16]
                l[j] = pp if l[j] is None else l[j] + pp
                probs[(j, cm)] = p
            p = probs[(j, cm)]
            if c < 2:
                return jnp.where(d > -16 * cm, p, 0.0)
            if c >= 16:
                return jnp.where(d > -16 * cm, 0.0, p)
            return p

        o = [None] * 4
        for kb in range(max(t - 2, 0), t + 1):
            rows = [[None] * 8 for _ in range(4)]
            for c in reversed(range(8)):
                xs = _regroup([prob(j, kb * 128 + c * 16) for j in range(4)], lane)
                for h in range(4):
                    rows[h][c] = xs[h]
            for h in range(4):
                p = jnp.concatenate(rows[h], axis=0).astype(bf16)
                vt = pltpu.bitcast(vt_ref[kb, h * 16:(h + 1) * 16, :], bf16)
                part = jnp.dot(vt, p, preferred_element_type=f32)
                o[h] = part if o[h] is None else o[h] + part
        inv = _regroup(
            [1.0 / jnp.sum(l[j], axis=0, keepdims=True) for j in range(4)], lane[0:1])
        ot = jnp.concatenate([o[h] * inv[h] for h in range(4)], axis=0).T
        out = _regroup([ot[32 * s:32 * s + 32] for s in range(4)],
                       lax.broadcasted_iota(jnp.int32, (32, 128), 1))
        o_ref[g, t * 128:(t + 1) * 128, :] = jnp.concatenate(out, axis=0).astype(bf16)

    def layer(li, carry):
        first = li == 0
        zero = (li >> 1).astype(u32)

        @pl.when(first)
        def _():
            x_copy(0).start()
            for cp in head_copies:
                cp.start()
            for c in range(1, nrc):
                x_copy(c).start()
            x_copy(0).wait()

        for j in range(8):
            ln_piece(0, j, 0)

        @pl.when(first)
        def _():
            for cp in head_copies:
                cp.wait()
            for cp in rest_copies:
                cp.start()

        def norm_body(c, _):
            for i in range(1, nrc):
                @pl.when(jnp.logical_and(first, c == i))
                def _():
                    x_copy(i).wait()

            for b in range(RC // 128):
                blk = c * (RC // 128) + b
                toks = [None]
                for part, pieces in ((2, (0, 1, 2)), (0, (3, 4, 5)), (1, (6, 7))):
                    project(part, 0, blk, cur_ref[b % 2], toks[-1])
                    lns = [ln_piece(jnp.minimum(blk + 1, NT - 1), j, (b + 1) % 2)
                           for j in pieces]
                    toks.append(_token(lns, zero))
            return _

        lax.fori_loop(0, nrc, norm_body, None)

        @pl.when(first)
        def _():
            for cp in late_copies:
                cp.start()
            for cp in rest_copies:
                cp.wait()

        def att_body(g, _):
            def nxt(part, blk):
                if 0 <= blk < NT:
                    project(part, g + 1, blk, xn_ref[blk * 128:(blk + 1) * 128, :])

            scores(0)
            nxt(0, 0)
            for t in range(NT + 2):
                if t + 1 < NT:
                    scores(t + 1)
                nxt(0, t + 1)
                nxt(1, t - 1)
                if t < NT:
                    attend(g, t)
                nxt(2, t - 2)
            return _

        lax.fori_loop(0, NG - 1, att_body, None)

        @pl.when(first)
        def _():
            for cp in late_copies:
                cp.wait()

        wr = wr_ref[...].astype(f32).reshape(1, D)
        best = jnp.full((8, 1), -jnp.inf, f32)
        best_i = jnp.zeros((8, 1), jnp.int32)
        sub = lax.broadcasted_iota(jnp.int32, (8, 1), 0)
        toks = [None, None]
        scores(0)
        scores(1)
        attend(NG - 1, 0)
        for t in range(NT + 1):
            for j in range(8):
                if j == 0 and t + 2 < NT:
                    scores(t + 2)
                if j == 3 and t + 1 < NT:
                    attend(NG - 1, t + 1)
                if t < NT:
                    o = jnp.concatenate(
                        [o_ref[g, t * 128:(t + 1) * 128, :] for g in range(NG)], axis=1)
                    w = _after(wo_ref[:, j * 128:(j + 1) * 128], toks[-2])
                    a_ref[t % 3, :, j * 128:(j + 1) * 128] = jnp.dot(
                        o, w, preferred_element_type=f32)
                if t > 0:
                    r0 = (t - 1) * 128 + j * 16
                    x1 = (x_ref[r0:r0 + 16, :].astype(f32)
                          + a_ref[(t - 1) % 3, j * 16:(j + 1) * 16, :])
                    ln = _layernorm(x1)
                    r = jnp.sum(ln * wr, axis=-1, keepdims=True)
                    x2 = x1 + ln
                    xn_ref[r0:r0 + 16, :] = ln.astype(bf16)
                    x_ref[r0:r0 + 16, :] = x2.astype(bf16)
                    for i in range(2):
                        ri = r[8 * i:8 * i + 8]
                        take = ri > best
                        best = jnp.where(take, ri, best)
                        best_i = jnp.where(take, sub + (r0 + 8 * i), best_i)
                    toks.append(_token([x2, jnp.broadcast_to(best, (8, 128))], zero))
            if t > 0 and (t * 128) % OUT_ROWS == 0:
                out_copy(t * 128 // OUT_ROWS - 1, t * 128 - OUT_ROWS, OUT_ROWS).start()

        top = jnp.max(best, axis=0, keepdims=True)
        idx = jnp.min(jnp.where(best == top, best_i, S - 1))
        base = pl.multiple_of((idx >> 4) << 4, 16)
        tile = pl.ds(base, 16)
        xs = xn_ref[tile, :]
        gate = jnp.dot(xs, wg_ref[...], preferred_element_type=f32)
        up = jnp.dot(xs, wu_ref[...], preferred_element_type=f32)
        hid = (gate * jax.nn.sigmoid(gate) * up).astype(bf16)
        y = None
        for j in range(F // 512):
            part = jnp.dot(hid[:, j * 512:(j + 1) * 512], wd_ref[j * 512:(j + 1) * 512, :],
                           preferred_element_type=f32)
            y = part if y is None else y + part
        y = y * jax.nn.sigmoid(top)
        xt = x_ref[tile, :].astype(f32)
        hit = lax.broadcasted_iota(jnp.int32, (16, D), 0) == idx - base
        new = jnp.where(hit, xt + y, xt).astype(bf16)
        for i in range(S // OUT_ROWS):
            out_copy(i, i * OUT_ROWS, OUT_ROWS).wait()
        x_ref[tile, :] = new

        @pl.when(jnp.logical_not(first))
        def _():
            fix = out_copy(0, base, 16)
            fix.start()
            fix.wait()

        return carry

    lax.fori_loop(0, 2, layer, None)


@jax.jit
def pallas_interleave_layers__sliding_block__moe_arch_mod__prompt_kernel(
    A_x: jax.Array,
    A_wqkv: jax.Array,
    A_wo: jax.Array,
    B_x: jax.Array,
    B_w_r: jax.Array,
    B_w_gate: jax.Array,
    B_w_up: jax.Array,
    B_w_down: jax.Array,
):
    del B_x
    hbm = pl.BlockSpec(memory_space=pl.ANY)
    return pl.pallas_call(
        _kernel,
        out_shape=jax.ShapeDtypeStruct((1, S, D), bf16),
        in_specs=[hbm, hbm, hbm, pl.BlockSpec(memory_space=pltpu.VMEM), hbm, hbm, hbm],
        out_specs=hbm,
        scratch_shapes=[
            pltpu.VMEM((S, D), bf16),
            pltpu.VMEM((S, D), bf16),
            pltpu.VMEM((NT, 64, 128), u32),
            pltpu.VMEM((NT, 64, 128), u32),
            pltpu.VMEM((NT, 64, 128), u32),
            pltpu.VMEM((NG, S, 128), bf16),
            pltpu.VMEM((D, 3 * D), bf16),
            pltpu.VMEM((D, D), bf16),
            pltpu.VMEM((D, F), bf16),
            pltpu.VMEM((D, F), bf16),
            pltpu.VMEM((F, D), bf16),
            pltpu.VMEM((2, 4, 256, 128), f32),
            pltpu.VMEM((2, 4, 8, 128), f32),
            pltpu.VMEM((2, 128, D), bf16),
            pltpu.VMEM((3, 128, D), f32),
            pltpu.SemaphoreType.DMA((S // RC,)),
            pltpu.SemaphoreType.DMA((10,)),
            pltpu.SemaphoreType.DMA((S // OUT_ROWS,)),
        ],
        compiler_params=pltpu.CompilerParams(vmem_limit_bytes=100 * 2**20),
    )(A_x, A_wqkv, A_wo, B_w_r, B_w_gate, B_w_up, B_w_down)
```

```python
import jax
import jax.numpy as jnp
from jax import lax
import jax.experimental.pallas as pl
import jax.experimental.pallas.tpu as pltpu

S = 2048
D = 1024
F = 3584
DH = 32
NG = D // 128
NT = S // 128
RC = 512
EPS = 1e-5
NEG = -1e9
LOG2E = 1.4426950408889634
SCALE = 0.1767578125
X_EDGES = (0, 640, 1152, 1664, 2048)
EARLY = 2
LAG = 3
OUT_ROWS = 256

bf16 = jnp.bfloat16
f32 = jnp.float32
u32 = jnp.uint32


def _round_bf16(v):
    return v.astype(bf16).astype(f32)


def _lane_moments(x):
    tiles = [x[:, j * 128:(j + 1) * 128] for j in range(D // 128)]
    mu = sum(tiles[1:], tiles[0]) * (128.0 / D)
    sq = [(t - mu) * (t - mu) for t in tiles]
    return mu, sum(sq[1:], sq[0])


def _row_stats(mu, m2):
    m = jnp.sum(mu, axis=-1, keepdims=True) * (1.0 / 128)
    e = mu - m
    v = jnp.sum(m2 + (D // 128) * (e * e), axis=-1, keepdims=True) * (1.0 / D)
    s = _round_bf16(jnp.sqrt(_round_bf16(_round_bf16(v) + EPS)))
    return _round_bf16(m), 1.0 / s


def _token(vals, zero):
    acc = None
    for v in vals:
        b = pltpu.bitcast(v, u32)
        for i in range(b.shape[0] // 8):
            for j in range(b.shape[1] // 128):
                t = b[8 * i:8 * i + 8, 128 * j:128 * j + 128]
                acc = t if acc is None else acc | t
    return acc & zero


def _after(b, tokens):
    parts = []
    half = b.shape[0] // 2
    for i in range(2):
        lo = i * half
        if i < len(tokens) and tokens[i] is not None:
            parts += [b[lo:lo + 8] | tokens[i], b[lo + 8:lo + half]]
        else:
            parts.append(b[lo:lo + half])
    return pltpu.bitcast(jnp.concatenate(parts, axis=0), bf16)


def _regroup(xs, lane):
    def sel(c, a, b):
        if a is None and b is None:
            return None
        return jnp.where(c, 0.0 if a is None else a, 0.0 if b is None else b)

    for bit in (1, 2):
        c = (lane & (32 * bit)) != 0
        xs = [sel(c, xs[h ^ bit], xs[h]) for h in range(4)]
    return xs


def _kernel(x_hbm, wqkv_hbm, wo_hbm, wr_ref, wg_hbm, wu_hbm, wd_hbm, out_hbm,
            x_ref, xn_ref, x1_ref, q_ref, k_ref, vt_ref, o_ref,
            wqkv_ref, wo_ref, wg_ref, wu_ref, wd_ref,
            s_ref, m_ref, pv_ref, wcur_ref, cur_ref, wr_rows, x_sem, w_sem, out_sem):
    nrc = S // RC

    def x_copy(c):
        rows = pl.ds(X_EDGES[c], X_EDGES[c + 1] - X_EDGES[c])
        return pltpu.make_async_copy(x_hbm.at[0, rows], x_ref.at[rows], x_sem.at[c])

    def wqkv_copy(part, lo, hi, sem):
        cols = pl.ds(part * D + lo, hi - lo)
        return pltpu.make_async_copy(
            wqkv_hbm.at[:, cols], wqkv_ref.at[:, cols], w_sem.at[sem])

    head_copies = [wqkv_copy(i, 0, 128, i) for i in range(3)]
    rest_copies = [wqkv_copy(i, 128, D, 3 + i) for i in range(3)]
    late_copies = [
        pltpu.make_async_copy(src, dst, w_sem.at[6 + i])
        for i, (src, dst) in enumerate(
            [(wo_hbm, wo_ref), (wg_hbm, wg_ref), (wu_hbm, wu_ref), (wd_hbm, wd_ref)])]

    def out_copy(i, r0, n):
        rows = pl.ds(r0, n)
        return pltpu.make_async_copy(x_ref.at[rows], out_hbm.at[0, rows], out_sem.at[i])

    def ln_piece(blk, j, slot, zero):
        rows = pl.ds(pl.multiple_of(blk * 128 + j * 16, 16), 16)
        shift, scale = _row_stats(*_lane_moments(x_ref[rows, :].astype(f32)))
        rows = pl.ds(pl.multiple_of((blk + zero) * 128 + j * 16, 16), 16)
        ln = (x_ref[rows, :].astype(f32) - shift) * scale
        xn = pltpu.bitcast(ln.astype(bf16), u32)
        xn_ref[pl.ds(pl.multiple_of(blk * 64 + j * 8, 8), 8), :] = xn
        cur_ref[slot, j * 8:(j + 1) * 8, :] = xn
        return xn

    def stage_weights(g):
        for part in range(3):
            cols = pl.ds(pl.multiple_of(part * D + g * 128, 128), 128)
            wcur_ref[part] = pltpu.bitcast(wqkv_ref[:, cols], u32)

    def project(part, blk, xn, tokens=()):
        y = jnp.dot(pltpu.bitcast(xn, bf16), _after(wcur_ref[part], tokens),
                    preferred_element_type=f32)
        if part == 0:
            y = y * (SCALE * LOG2E)
        if part == 2:
            y = y.T
        (q_ref, k_ref, vt_ref)[part][blk] = pltpu.bitcast(y.astype(bf16), u32)

    def tri():
        return (lax.broadcasted_iota(jnp.int32, (16, 128), 0)
                - (lax.broadcasted_iota(jnp.int32, (16, 128), 1) & 31))

    def scores(t):
        slot = t % 2
        head = lax.broadcasted_iota(jnp.int32, (16, 128), 1) >> 5
        tiles = []
        for j in range(4):
            k0 = t * 128 + j * 32 - 256
            order = [c for c in [0, 16, 1, 17] + list(range(2, 16)) if k0 + 16 * c >= 0]
            parts = []
            for c in order:
                key = k0 + 16 * c
                parts.append(k_ref[key // 128, key % 128 // 2:key % 128 // 2 + 8, :])
            kw = pltpu.bitcast(jnp.concatenate(parts, axis=0), bf16)
            qt = q_ref[t, j * 16:(j + 1) * 16, :]
            w = jnp.concatenate(
                [jnp.where(head == (s ^ j), qt, jnp.zeros_like(qt)) for s in range(4)],
                axis=0)
            sc = lax.dot_general(kw, pltpu.bitcast(w, bf16), (((1,), (1,)), ((), ())),
                                 preferred_element_type=f32)
            tiles.append({c: sc[16 * i:16 * i + 16] for i, c in enumerate(order)})
        d = tri()
        ms = [None] * 4
        for c in range(16):
            for j in range(4):
                if c < 2:
                    sm = jnp.where(d > -16 * c, tiles[j].get(c, NEG), tiles[j][c + 16])
                elif c in tiles[j]:
                    sm = tiles[j][c]
                else:
                    continue
                s_ref[slot, j, 16 * c:16 * c + 16, :] = sm
                mm = jnp.maximum(sm[0:8], sm[8:16])
                ms[j] = mm if ms[j] is None else jnp.maximum(ms[j], mm)
        for j in range(4):
            m_ref[slot, j] = jnp.broadcast_to(
                jnp.max(ms[j], axis=0, keepdims=True), (8, 128))

    def attend(g, t):
        slot = t % 2
        d = tri()
        lane = lax.broadcasted_iota(jnp.int32, (16, 128), 1)
        m2 = [jnp.concatenate([m_ref[slot, j]] * 2, axis=0) for j in range(4)]
        l = [None] * 4
        probs = {}

        def prob(j, key):
            c = (key - (t * 128 + j * 32 - 256)) // 16
            if c < 0 or c >= 18:
                return None
            cm = c % 16
            if (j, cm) not in probs:
                p = jnp.exp2(s_ref[slot, j, 16 * cm:16 * cm + 16, :] - m2[j])
                pp = p[0:8] + p[8:16]
                l[j] = pp if l[j] is None else l[j] + pp
                probs[(j, cm)] = p
            p = probs[(j, cm)]
            if c < 2:
                return jnp.where(d > -16 * cm, p, 0.0)
            if c >= 16:
                return jnp.where(d > -16 * cm, 0.0, p)
            return p

        o = [None] * 4
        for kb in range(t - 2, t + 1):
            if kb > t - 2:
                yield
            if kb < 0:
                continue
            rows = [[None] * 8 for _ in range(4)]
            for c in reversed(range(8)):
                xs = _regroup([prob(j, kb * 128 + c * 16) for j in range(4)], lane)
                for h in range(4):
                    rows[h][c] = xs[h]
            for h in range(4):
                p = jnp.concatenate(rows[h], axis=0).astype(bf16)
                vt = pltpu.bitcast(vt_ref[kb, h * 16:(h + 1) * 16, :], bf16)
                part = jnp.dot(vt, p, preferred_element_type=f32)
                if kb < t:
                    pv_ref[t - 1 - kb, h] = part
                else:
                    for i in range(min(t, 2)):
                        part = part + pv_ref[i, h]
                    o[h] = part
        inv = _regroup(
            [1.0 / jnp.sum(l[j], axis=0, keepdims=True) for j in range(4)], lane[0:1])
        ot = jnp.concatenate([o[h] * inv[h] for h in range(4)], axis=0).T
        out = _regroup([ot[32 * s:32 * s + 32] for s in range(4)],
                       lax.broadcasted_iota(jnp.int32, (32, 128), 1))
        o_ref[g, t] = pltpu.bitcast(jnp.concatenate(out, axis=0).astype(bf16), u32)
        yield

    def layer(li, carry):
        first = li == 0
        izero = li >> 1
        zero = izero.astype(u32)

        @pl.when(first)
        def _():
            x_copy(0).start()
            for cp in head_copies:
                cp.start()
            x_copy(0).wait()
            for cp in head_copies:
                cp.wait()
            for c in range(1, nrc):
                x_copy(c).start()
            for cp in rest_copies:
                cp.start()

        stage_weights(0)
        for j in range(8):
            ln_piece(0, j, 0, izero)

        def norm_body(c, _):
            for i in range(1, nrc):
                @pl.when(jnp.logical_and(first, c == i))
                def _():
                    x_copy(i).wait()

            for b in range(RC // 128):
                blk = c * (RC // 128) + b
                lns = [ln_piece(jnp.minimum(blk + 1, NT - 1), j, (b + 1) % 2, izero)
                       for j in range(8)]
                toks = [None] + [_token([lns[j] for j in js], zero)
                                 for js in ((0,), (1, 2), (3,), (4, 5), (6,))]
                for i, part in enumerate((2, 0, 1)):
                    project(part, blk, cur_ref[b % 2], toks[2 * i:2 * i + 2])
            return _

        lax.fori_loop(0, nrc, norm_body, None)

        @pl.when(first)
        def _():
            for cp in late_copies:
                cp.start()
            for cp in rest_copies:
                cp.wait()

        def att_body(g, _):
            def nxt(part, blk):
                if 0 <= blk < NT:
                    project(part, blk, xn_ref[blk * 64:(blk + 1) * 64, :])

            stage_weights(g + 1)
            scores(0)
            for t in range(NT):
                if t + 1 < NT:
                    scores(t + 1)
                steps = attend(g, t)
                for part in range(3):
                    nxt(part, t - part)
                    next(steps)
            nxt(2, NT - 2)
            nxt(2, NT - 1)
            nxt(1, NT - 1)
            return _

        lax.fori_loop(0, NG - 1, att_body, None)

        @pl.when(first)
        def _():
            for cp in late_copies:
                cp.wait()

        stats = {}
        wr_sum = jnp.sum(wr_rows[...], axis=-1, keepdims=True)
        best = jnp.full((8, 1), -jnp.inf, f32)
        best_i = jnp.zeros((8, 1), jnp.int32)
        sub = lax.broadcasted_iota(jnp.int32, (8, 1), 0)
        toks = [None] * 8
        scores(0)
        for t in range(NT):
            if t + 1 < NT:
                scores(t + 1)
            steps = attend(NG - 1, t)
            o = pltpu.bitcast(jnp.concatenate(
                [o_ref[g, t] for g in range(EARLY)], axis=1), bf16)
            for j in range(4):
                blk = (slice(t * 128, (t + 1) * 128), slice(j * 256, (j + 1) * 256))
                x1_ref[blk] = x_ref[blk].astype(f32) + jnp.dot(
                    o, wo_ref[0:EARLY * 128, blk[1]], preferred_element_type=f32)
                if j < 3:
                    next(steps)
        for t in range(NT + 1):
            for j in range(8):
                if t < NT:
                    o = pltpu.bitcast(jnp.concatenate(
                        [o_ref[g, t] for g in range(EARLY, NG)], axis=1), bf16)
                    w = _after(pltpu.bitcast(wo_ref[EARLY * 128:, j * 128:(j + 1) * 128], u32),
                               [toks[-6]])
                    a = jnp.dot(o, w, preferred_element_type=f32)
                    blk = (slice(t * 128, (t + 1) * 128), slice(j * 128, (j + 1) * 128))
                    x1_ref[blk] = a + x1_ref[blk]
                    go = _token([a[0:8]], zero)
                done = []
                p = (t - 1) * 8 + j
                if t > 0:
                    x1 = pltpu.bitcast(x1_ref[p * 16:(p + 1) * 16, :], u32)
                    x1 = pltpu.bitcast(x1 | jnp.tile(go, (2, D // 128)), f32)
                    moments = _lane_moments(x1)
                    shift, scale = _row_stats(*moments)
                    xw = jnp.sum(x1 * wr_rows[...], axis=-1, keepdims=True)
                    stats[p] = (1.0 + scale, shift * scale, (xw - shift * wr_sum) * scale)
                    done += moments
                last = p == S // 16 - 1
                for f in range(max(p - LAG, 0), p + 1 if last else p - LAG + 1):
                    r0 = f * 16
                    gain, offset, r = stats[f]
                    rows = pl.ds(pl.multiple_of(izero * 16 + r0, 16), 16)
                    x2 = (x1_ref[rows, :] * gain - offset).astype(bf16)
                    x_ref[r0:r0 + 16, :] = x2
                    for i in range(2):
                        ri = r[8 * i:8 * i + 8]
                        take = ri > best
                        best = jnp.where(take, ri, best)
                        best_i = jnp.where(take, sub + (r0 + 8 * i), best_i)
                    done += [jnp.broadcast_to(best, (8, 128))]
                    if (r0 + 16) % OUT_ROWS == 0:
                        out_copy(r0 // OUT_ROWS, r0 + 16 - OUT_ROWS, OUT_ROWS).start()
                toks.append(_token(done, zero) if done else None)

        top = jnp.max(best, axis=0, keepdims=True)
        idx = jnp.min(jnp.where(best == top, best_i, S - 1))
        base = pl.multiple_of((idx >> 4) << 4, 16)
        tile = pl.ds(base, 16)
        x1 = x1_ref[tile, :]
        shift, scale = _row_stats(*_lane_moments(x1))
        ln = (x1 - shift) * scale
        xs = ln.astype(bf16)
        gate = jnp.dot(xs, wg_ref[...], preferred_element_type=f32)
        up = jnp.dot(xs, wu_ref[...], preferred_element_type=f32)
        hid = (gate * jax.nn.sigmoid(gate) * up).astype(bf16)
        y = None
        for j in range(F // 512):
            part = jnp.dot(hid[:, j * 512:(j + 1) * 512], wd_ref[j * 512:(j + 1) * 512, :],
                           preferred_element_type=f32)
            y = part if y is None else y + part
        y = y * jax.nn.sigmoid(top)
        xt = x_ref[tile, :].astype(f32)
        hit = lax.broadcasted_iota(jnp.int32, (16, D), 0) == idx - base
        new = jnp.where(hit, x1 + ln + y, xt).astype(bf16)
        for i in range(S // OUT_ROWS):
            out_copy(i, i * OUT_ROWS, OUT_ROWS).wait()
        x_ref[tile, :] = new

        @pl.when(jnp.logical_not(first))
        def _():
            fix = out_copy(0, base, 16)
            fix.start()
            fix.wait()

        return carry

    wr_rows[...] = jnp.broadcast_to(wr_ref[...].astype(f32).reshape(1, D), (16, D))
    lax.fori_loop(0, 2, layer, None)


@jax.jit
def pallas_interleave_layers__sliding_block__moe_arch_mod__prompt_kernel(
    A_x: jax.Array,
    A_wqkv: jax.Array,
    A_wo: jax.Array,
    B_x: jax.Array,
    B_w_r: jax.Array,
    B_w_gate: jax.Array,
    B_w_up: jax.Array,
    B_w_down: jax.Array,
):
    del B_x
    hbm = pl.BlockSpec(memory_space=pl.ANY)
    return pl.pallas_call(
        _kernel,
        out_shape=jax.ShapeDtypeStruct((1, S, D), bf16),
        in_specs=[hbm, hbm, hbm, pl.BlockSpec(memory_space=pltpu.VMEM), hbm, hbm, hbm],
        out_specs=hbm,
        scratch_shapes=[
            pltpu.VMEM((S, D), bf16),
            pltpu.VMEM((S // 2, D), u32),
            pltpu.VMEM((S, D), f32),
            pltpu.VMEM((NT, 64, 128), u32),
            pltpu.VMEM((NT, 64, 128), u32),
            pltpu.VMEM((NT, 64, 128), u32),
            pltpu.VMEM((NG, NT, 64, 128), u32),
            pltpu.VMEM((D, 3 * D), bf16),
            pltpu.VMEM((D, D), bf16),
            pltpu.VMEM((D, F), bf16),
            pltpu.VMEM((D, F), bf16),
            pltpu.VMEM((F, D), bf16),
            pltpu.VMEM((2, 4, 256, 128), f32),
            pltpu.VMEM((2, 4, 8, 128), f32),
            pltpu.VMEM((2, 4, 32, 128), f32),
            pltpu.VMEM((3, D // 2, 128), u32),
            pltpu.VMEM((2, 64, D), u32),
            pltpu.VMEM((16, D), f32),
            pltpu.SemaphoreType.DMA((S // RC,)),
            pltpu.SemaphoreType.DMA((10,)),
            pltpu.SemaphoreType.DMA((S // OUT_ROWS,)),
        ],
        compiler_params=pltpu.CompilerParams(vmem_limit_bytes=100 * 2**20),
    )(A_x, A_wqkv, A_wo, B_w_r, B_w_gate, B_w_up, B_w_down)
```

```python
import jax
import jax.numpy as jnp
from jax import lax
import jax.experimental.pallas as pl
import jax.experimental.pallas.tpu as pltpu

S = 2048
D = 1024
F = 3584
DH = 32
NG = D // 128
NT = S // 128
RC = 512
EPS = 1e-5
NEG = -1e9
LOG2E = 1.4426950408889634
SCALE = 0.1767578125
X_EDGES = (0, 256, 768, 1280, 1792, 2048)
EARLY = 2
APPLY_AT = ((), (0,), (1,), (2, 3), (4, 5), (6, 7))
STATS_AT = ((0, 1), (2, 3), (4, 5), (6, 7), (), ())
LAG = 3
OUT_ROWS = 256

bf16 = jnp.bfloat16
f32 = jnp.float32
u32 = jnp.uint32


def _round_bf16(v):
    return v.astype(bf16).astype(f32)


def _lane_moments(x):
    tiles = [x[:, j * 128:(j + 1) * 128] for j in range(D // 128)]
    mu = sum(tiles[1:], tiles[0]) * (128.0 / D)
    sq = [(t - mu) * (t - mu) for t in tiles]
    return mu, sum(sq[1:], sq[0])


def _row_moments(mu, m2):
    m = jnp.sum(mu, axis=-1, keepdims=True) * (1.0 / 128)
    e = mu - m
    return m, jnp.sum(m2 + (D // 128) * (e * e), axis=-1, keepdims=True) * (1.0 / D)


def _inv_std(v):
    return 1.0 / _round_bf16(jnp.sqrt(_round_bf16(_round_bf16(v) + EPS)))


def _row_stats(mu, m2):
    m, v = _row_moments(mu, m2)
    return _round_bf16(m), _inv_std(v)


def _token(vals, zero):
    acc = None
    for v in vals:
        b = pltpu.bitcast(v, u32)
        for i in range(b.shape[0] // 8):
            for j in range(b.shape[1] // 128):
                t = b[8 * i:8 * i + 8, 128 * j:128 * j + 128]
                acc = t if acc is None else acc | t
    return acc & zero


def _after(b, tokens):
    parts = []
    half = b.shape[0] // 2
    for i in range(2):
        lo = i * half
        if i < len(tokens) and tokens[i] is not None:
            parts += [b[lo:lo + 8] | tokens[i], b[lo + 8:lo + half]]
        else:
            parts.append(b[lo:lo + half])
    return pltpu.bitcast(jnp.concatenate(parts, axis=0), bf16)


def _regroup(xs, lane):
    def sel(c, a, b):
        if a is None and b is None:
            return None
        return jnp.where(c, 0.0 if a is None else a, 0.0 if b is None else b)

    for bit in (1, 2):
        c = (lane & (32 * bit)) != 0
        xs = [sel(c, xs[h ^ bit], xs[h]) for h in range(4)]
    return xs


def _kernel(x_hbm, wqkv_hbm, wo_hbm, wr_hbm, wg_hbm, wu_hbm, wd_hbm, out_hbm,
            x_ref, xn_ref, x1_ref, q_ref, k_ref, vt_ref, o_ref,
            wqkv_ref, wo_ref, wg_ref, wu_ref, wd_ref,
            s_ref, m_ref, pv_ref, wcur_ref, cur_ref, shift_ref, var_ref, wr_ref, wr_rows, x_sem, w_sem, out_sem):
    nrc = S // RC

    def x_copy(c):
        rows = pl.ds(X_EDGES[c], X_EDGES[c + 1] - X_EDGES[c])
        return pltpu.make_async_copy(x_hbm.at[0, rows], x_ref.at[rows], x_sem.at[c])

    def wqkv_copy(part, lo, hi, sem):
        cols = pl.ds(part * D + lo, hi - lo)
        return pltpu.make_async_copy(
            wqkv_hbm.at[:, cols], wqkv_ref.at[:, cols], w_sem.at[sem])

    head_copies = [wqkv_copy(i, 0, 128, i) for i in range(3)]
    next_copies = [wqkv_copy(i, 128, 256, 3 + i) for i in range(3)]
    rest_copies = [wqkv_copy(i, 256, D, 6 + i) for i in range(3)]
    wr_copy = pltpu.make_async_copy(wr_hbm, wr_ref, w_sem.at[9])
    late_copies = [
        pltpu.make_async_copy(src, dst, w_sem.at[10 + i])
        for i, (src, dst) in enumerate(
            [(wo_hbm, wo_ref), (wg_hbm, wg_ref), (wu_hbm, wu_ref), (wd_hbm, wd_ref)])]

    def out_copy(i, r0, n):
        rows = pl.ds(r0, n)
        return pltpu.make_async_copy(x_ref.at[rows], out_hbm.at[0, rows], out_sem.at[i])

    def load_rows(blk, j, go):
        x = x_ref[pl.ds(pl.multiple_of(blk * 128 + j * 16, 16), 16), :].astype(f32)
        if go is None:
            return x
        first = pltpu.bitcast(x[:, 0:128], u32) | jnp.concatenate([go, go], axis=0)
        return jnp.concatenate([pltpu.bitcast(first, f32), x[:, 128:]], axis=1)

    def ln_stats(blk, j, slot, go=None):
        m, v = _row_moments(*_lane_moments(load_rows(blk, j, go)))
        shift_ref[slot, j * 16:(j + 1) * 16, :] = jnp.broadcast_to(
            _round_bf16(m), (16, 128))
        v = jnp.broadcast_to(v, (16, 128))
        return [v[0:8], v[8:16]]

    def ln_gather(slot, vs):
        lane = lax.broadcasted_iota(jnp.int32, (8, 128), 1)
        bit = 1
        while len(vs) > 1:
            vs = [jnp.where((lane & bit) != 0, vs[i + 1], vs[i])
                  for i in range(0, len(vs), 2)]
            bit *= 2
        var_ref[slot] = vs[0]

    def ln_apply(blk, j, slot, scales, go=None):
        shift = shift_ref[slot, j * 16:(j + 1) * 16, :]
        if go is not None:
            shift = pltpu.bitcast(
                pltpu.bitcast(shift, u32) | jnp.concatenate([go, go], axis=0), f32)
        scale = jnp.concatenate(
            [jnp.broadcast_to(scales[:, i:i + 1], (8, 128)) for i in (2 * j, 2 * j + 1)],
            axis=0)
        ln = ((load_rows(blk, j, None) - jnp.tile(shift, (1, D // 128)))
              * jnp.tile(scale, (1, D // 128)))
        cur_ref[slot, j * 16:(j + 1) * 16, :] = ln.astype(bf16)

    def stage_weights(g):
        for part in range(3):
            cols = pl.ds(pl.multiple_of(part * D + g * 128, 128), 128)
            wcur_ref[part] = pltpu.bitcast(wqkv_ref[:, cols], u32)

    def project(part, blk, xn, tokens=()):
        y = jnp.dot(pltpu.bitcast(xn, bf16), _after(wcur_ref[part], tokens),
                    preferred_element_type=f32)
        marks = (y[0:8], y[64:72])
        if part == 0:
            y = y * (SCALE * LOG2E)
        if part == 2:
            y = y.T
        (q_ref, k_ref, vt_ref)[part][blk] = pltpu.bitcast(y.astype(bf16), u32)
        return marks

    def tri():
        return (lax.broadcasted_iota(jnp.int32, (16, 128), 0)
                - (lax.broadcasted_iota(jnp.int32, (16, 128), 1) & 31))

    def scores(t):
        slot = t % 2
        head = lax.broadcasted_iota(jnp.int32, (16, 128), 1) >> 5
        tiles = []
        for j in range(4):
            k0 = t * 128 + j * 32 - 256
            order = [c for c in [0, 16, 1, 17] + list(range(2, 16)) if k0 + 16 * c >= 0]
            parts = []
            for c in order:
                key = k0 + 16 * c
                parts.append(k_ref[key // 128, key % 128 // 2:key % 128 // 2 + 8, :])
            kw = pltpu.bitcast(jnp.concatenate(parts, axis=0), bf16)
            qt = q_ref[t, j * 16:(j + 1) * 16, :]
            w = jnp.concatenate(
                [jnp.where(head == (s ^ j), qt, jnp.zeros_like(qt)) for s in range(4)],
                axis=0)
            sc = lax.dot_general(kw, pltpu.bitcast(w, bf16), (((1,), (1,)), ((), ())),
                                 preferred_element_type=f32)
            tiles.append({c: sc[16 * i:16 * i + 16] for i, c in enumerate(order)})
        d = tri()
        ms = [None] * 4
        for c in range(16):
            for j in range(4):
                if c < 2:
                    sm = jnp.where(d > -16 * c, tiles[j].get(c, NEG), tiles[j][c + 16])
                elif c in tiles[j]:
                    sm = tiles[j][c]
                else:
                    continue
                s_ref[slot, j, 16 * c:16 * c + 16, :] = sm
                mm = jnp.maximum(sm[0:8], sm[8:16])
                ms[j] = mm if ms[j] is None else jnp.maximum(ms[j], mm)
        for j in range(4):
            m_ref[slot, j] = jnp.broadcast_to(
                jnp.max(ms[j], axis=0, keepdims=True), (8, 128))

    def attend(g, t):
        slot = t % 2
        d = tri()
        lane = lax.broadcasted_iota(jnp.int32, (16, 128), 1)
        m2 = [jnp.concatenate([m_ref[slot, j]] * 2, axis=0) for j in range(4)]
        l = [None] * 4
        probs = {}

        def prob(j, key):
            c = (key - (t * 128 + j * 32 - 256)) // 16
            if c < 0 or c >= 18:
                return None
            cm = c % 16
            if (j, cm) not in probs:
                p = jnp.exp2(s_ref[slot, j, 16 * cm:16 * cm + 16, :] - m2[j])
                pp = p[0:8] + p[8:16]
                l[j] = pp if l[j] is None else l[j] + pp
                probs[(j, cm)] = p
            p = probs[(j, cm)]
            if c < 2:
                return jnp.where(d > -16 * cm, p, 0.0)
            if c >= 16:
                return jnp.where(d > -16 * cm, 0.0, p)
            return p

        o = [None] * 4
        for kb in range(t - 2, t + 1):
            if kb > t - 2:
                yield
            if kb < 0:
                continue
            rows = [[None] * 8 for _ in range(4)]
            for c in reversed(range(8)):
                xs = _regroup([prob(j, kb * 128 + c * 16) for j in range(4)], lane)
                for h in range(4):
                    rows[h][c] = xs[h]
            for h in range(4):
                p = jnp.concatenate(rows[h], axis=0).astype(bf16)
                vt = pltpu.bitcast(vt_ref[kb, h * 16:(h + 1) * 16, :], bf16)
                part = jnp.dot(vt, p, preferred_element_type=f32)
                if kb < t:
                    pv_ref[t - 1 - kb, h] = part
                else:
                    for i in range(min(t, 2)):
                        part = part + pv_ref[i, h]
                    o[h] = part
        inv = _regroup(
            [1.0 / jnp.sum(l[j], axis=0, keepdims=True) for j in range(4)], lane[0:1])
        ot = jnp.concatenate([o[h] * inv[h] for h in range(4)], axis=0).T
        out = _regroup([ot[32 * s:32 * s + 32] for s in range(4)],
                       lax.broadcasted_iota(jnp.int32, (32, 128), 1))
        o_ref[g, t] = pltpu.bitcast(jnp.concatenate(out, axis=0).astype(bf16), u32)
        yield

    def layer(li, carry):
        first = li == 0
        izero = li >> 1
        zero = izero.astype(u32)

        @pl.when(first)
        def _():
            x_copy(0).start()
            wr_copy.start()
            for cp in head_copies:
                cp.start()
            x_copy(1).start()
            wr_copy.wait()
            wr_rows[...] = jnp.broadcast_to(
                wr_ref[...].astype(f32).reshape(1, D), (16, D))
            x_copy(0).wait()

        for blk in range(2):
            ln_gather(blk, [v for j in range(8) for v in ln_stats(blk, j, blk)])
        scales = _inv_std(var_ref[0])
        for j in range(8):
            ln_apply(izero, j, 0, scales)

        @pl.when(first)
        def _():
            for cp in head_copies:
                cp.wait()
            x_copy(2).start()

        stage_weights(0)

        def norm_body(c, _):
            for i in range(nrc):
                @pl.when(jnp.logical_and(first, c == i))
                def _():
                    x_copy(i + 1).wait()
                    if i + 3 < len(X_EDGES) - 1:
                        x_copy(i + 3).start()
                    for cp in ([], next_copies, rest_copies, [])[i]:
                        cp.start()

            go = [None, None]
            for b in range(RC // 128):
                blk = c * (RC // 128) + b
                xn = pltpu.bitcast(cur_ref[b % 2], u32)
                xn_ref[pl.ds(pl.multiple_of(blk * 64, 64), 64), :] = xn
                scales = _inv_std(var_ref[(b + 1) % 2])
                vs = []
                for i, part in enumerate((2, 0, 1)):
                    for h in range(2):
                        for j in APPLY_AT[2 * i + h]:
                            ln_apply(jnp.minimum(blk + 1, NT - 1), j, (b + 1) % 2,
                                     scales, go[h])
                        for j in STATS_AT[2 * i + h]:
                            vs += ln_stats(jnp.minimum(blk + 2, NT - 1), j, b % 2, go[h])
                    go = [_token([m], zero) for m in project(part, blk, xn)]
                ln_gather(b % 2, vs)
            return _

        lax.fori_loop(0, nrc, norm_body, None)

        @pl.when(first)
        def _():
            for cp in next_copies:
                cp.wait()

        def att_body(g, _):
            def nxt(part, blk):
                if 0 <= blk < NT:
                    project(part, blk, xn_ref[blk * 64:(blk + 1) * 64, :])

            @pl.when(jnp.logical_and(first, g == 1))
            def _():
                for cp in rest_copies:
                    cp.wait()
                for cp in late_copies:
                    cp.start()

            stage_weights(g + 1)
            scores(0)
            for t in range(NT):
                if t + 1 < NT:
                    scores(t + 1)
                steps = attend(g, t)
                for part in range(3):
                    nxt(part, t - part)
                    next(steps)
            nxt(2, NT - 2)
            nxt(2, NT - 1)
            nxt(1, NT - 1)
            return _

        lax.fori_loop(0, NG - 1, att_body, None)

        @pl.when(first)
        def _():
            for cp in late_copies:
                cp.wait()

        stats = {}
        wr_sum = jnp.sum(wr_rows[...], axis=-1, keepdims=True)
        best = jnp.full((8, 1), -jnp.inf, f32)
        best_i = jnp.zeros((8, 1), jnp.int32)
        sub = lax.broadcasted_iota(jnp.int32, (8, 1), 0)
        toks = [None] * 8
        scores(0)
        for t in range(NT):
            if t + 1 < NT:
                scores(t + 1)
            steps = attend(NG - 1, t)
            o = pltpu.bitcast(jnp.concatenate(
                [o_ref[g, t] for g in range(EARLY)], axis=1), bf16)
            for j in range(4):
                blk = (slice(t * 128, (t + 1) * 128), slice(j * 256, (j + 1) * 256))
                x1_ref[blk] = x_ref[blk].astype(f32) + jnp.dot(
                    o, wo_ref[0:EARLY * 128, blk[1]], preferred_element_type=f32)
                if j < 3:
                    next(steps)
        for t in range(NT + 1):
            for j in range(8):
                if t < NT:
                    o = pltpu.bitcast(jnp.concatenate(
                        [o_ref[g, t] for g in range(EARLY, NG)], axis=1), bf16)
                    w = _after(pltpu.bitcast(wo_ref[EARLY * 128:, j * 128:(j + 1) * 128], u32),
                               [toks[-6]])
                    a = jnp.dot(o, w, preferred_element_type=f32)
                    blk = (slice(t * 128, (t + 1) * 128), slice(j * 128, (j + 1) * 128))
                    x1_ref[blk] = a + x1_ref[blk]
                    go = _token([a[0:8]], zero)
                done = []
                p = (t - 1) * 8 + j
                if t > 0:
                    x1 = pltpu.bitcast(x1_ref[p * 16:(p + 1) * 16, :], u32)
                    x1 = pltpu.bitcast(x1 | jnp.tile(go, (2, D // 128)), f32)
                    moments = _lane_moments(x1)
                    shift, scale = _row_stats(*moments)
                    xw = jnp.sum(x1 * wr_rows[...], axis=-1, keepdims=True)
                    stats[p] = (1.0 + scale, shift * scale, (xw - shift * wr_sum) * scale)
                    done += moments
                last = p == S // 16 - 1
                for f in range(max(p - LAG, 0), p + 1 if last else p - LAG + 1):
                    r0 = f * 16
                    gain, offset, r = stats[f]
                    rows = pl.ds(pl.multiple_of(izero * 16 + r0, 16), 16)
                    x2 = (x1_ref[rows, :] * gain - offset).astype(bf16)
                    x_ref[r0:r0 + 16, :] = x2
                    for i in range(2):
                        ri = r[8 * i:8 * i + 8]
                        take = ri > best
                        best = jnp.where(take, ri, best)
                        best_i = jnp.where(take, sub + (r0 + 8 * i), best_i)
                    done += [jnp.broadcast_to(best, (8, 128))]
                    if (r0 + 16) % OUT_ROWS == 0:
                        out_copy(r0 // OUT_ROWS, r0 + 16 - OUT_ROWS, OUT_ROWS).start()
                toks.append(_token(done, zero) if done else None)

        top = jnp.max(best, axis=0, keepdims=True)
        idx = jnp.min(jnp.where(best == top, best_i, S - 1))
        base = pl.multiple_of((idx >> 4) << 4, 16)
        tile = pl.ds(base, 16)
        x1 = x1_ref[tile, :]
        shift, scale = _row_stats(*_lane_moments(x1))
        ln = (x1 - shift) * scale
        xs = ln.astype(bf16)
        gate = jnp.dot(xs, wg_ref[...], preferred_element_type=f32)
        up = jnp.dot(xs, wu_ref[...], preferred_element_type=f32)
        hid = (gate * jax.nn.sigmoid(gate) * up).astype(bf16)
        y = None
        weight = jax.nn.sigmoid(top)
        for j in range(F // 512):
            part = jnp.dot(hid[:, j * 512:(j + 1) * 512], wd_ref[j * 512:(j + 1) * 512, :],
                           preferred_element_type=f32) * weight
            y = part if y is None else y + part
        xt = x_ref[tile, :].astype(f32)
        hit = lax.broadcasted_iota(jnp.int32, (16, D), 0) == idx - base
        new = jnp.where(hit, x1 + ln + y, xt).astype(bf16)
        for i in range(S // OUT_ROWS):
            out_copy(i, i * OUT_ROWS, OUT_ROWS).wait()
        x_ref[tile, :] = new

        @pl.when(jnp.logical_not(first))
        def _():
            fix = out_copy(0, base, 16)
            fix.start()
            fix.wait()

        return carry

    lax.fori_loop(0, 2, layer, None)


@jax.jit
def pallas_interleave_layers__sliding_block__moe_arch_mod__prompt_kernel(
    A_x: jax.Array,
    A_wqkv: jax.Array,
    A_wo: jax.Array,
    B_x: jax.Array,
    B_w_r: jax.Array,
    B_w_gate: jax.Array,
    B_w_up: jax.Array,
    B_w_down: jax.Array,
):
    del B_x
    hbm = pl.BlockSpec(memory_space=pl.ANY)
    return pl.pallas_call(
        _kernel,
        out_shape=jax.ShapeDtypeStruct((1, S, D), bf16),
        in_specs=[hbm] * 7,
        out_specs=hbm,
        scratch_shapes=[
            pltpu.VMEM((S, D), bf16),
            pltpu.VMEM((S // 2, D), u32),
            pltpu.VMEM((S, D), f32),
            pltpu.VMEM((NT, 64, 128), u32),
            pltpu.VMEM((NT, 64, 128), u32),
            pltpu.VMEM((NT, 64, 128), u32),
            pltpu.VMEM((NG, NT, 64, 128), u32),
            pltpu.VMEM((D, 3 * D), bf16),
            pltpu.VMEM((D, D), bf16),
            pltpu.VMEM((D, F), bf16),
            pltpu.VMEM((D, F), bf16),
            pltpu.VMEM((F, D), bf16),
            pltpu.VMEM((2, 4, 256, 128), f32),
            pltpu.VMEM((2, 4, 8, 128), f32),
            pltpu.VMEM((2, 4, 32, 128), f32),
            pltpu.VMEM((3, D // 2, 128), u32),
            pltpu.VMEM((2, 128, D), bf16),
            pltpu.VMEM((2, 128, 128), f32),
            pltpu.VMEM((2, 8, 128), f32),
            pltpu.VMEM((D,), bf16),
            pltpu.VMEM((16, D), f32),
            pltpu.SemaphoreType.DMA((len(X_EDGES) - 1,)),
            pltpu.SemaphoreType.DMA((14,)),
            pltpu.SemaphoreType.DMA((S // OUT_ROWS,)),
        ],
        compiler_params=pltpu.CompilerParams(vmem_limit_bytes=100 * 2**20),
    )(A_x, A_wqkv, A_wo, B_w_r, B_w_gate, B_w_up, B_w_down)
```

```python
import jax
import jax.numpy as jnp
from jax import lax
import jax.experimental.pallas as pl
import jax.experimental.pallas.tpu as pltpu

S = 2048
D = 1024
F = 3584
NG = D // 128
NT = S // 128
RC = 512
EPS = 1e-5
NEG = -1e9
LOG2E = 1.4426950408889634
SCALE = 0.1767578125
X_EDGES = (0, 256, 768, 1280, 1792, 2048)
EARLY = 2
APPLY_AT = ((), (0,), (1,), (2, 3), (4, 5), (6, 7))
STATS_AT = ((0, 1), (2, 3), (4, 5), (6, 7), (), ())
LAG = 3
OUT_ROWS = 256

bf16 = jnp.bfloat16
f32 = jnp.float32
u32 = jnp.uint32


def _round_bf16(v):
    return v.astype(bf16).astype(f32)


def _widen(v):
    return jnp.concatenate([v] * (D // 128), axis=1)


def _lane_moments(x):
    tiles = [x[:, j * 128:(j + 1) * 128] for j in range(D // 128)]
    mu = sum(tiles[1:], tiles[0]) * (128.0 / D)
    sq = [(t - mu) * (t - mu) for t in tiles]
    return mu, sum(sq[1:], sq[0])


def _row_moments(mu, m2):
    m = jnp.sum(mu, axis=-1, keepdims=True) * (1.0 / 128)
    e = mu - m
    return m, jnp.sum(m2 + (D // 128) * (e * e), axis=-1, keepdims=True) * (1.0 / D)


def _inv_std(v):
    return 1.0 / _round_bf16(jnp.sqrt(_round_bf16(_round_bf16(v) + EPS)))


def _row_stats(mu, m2):
    m, v = _row_moments(mu, m2)
    return _round_bf16(m), _inv_std(v)


def _token(vals, zero):
    acc = None
    for v in vals:
        b = pltpu.bitcast(v, u32)
        for i in range(b.shape[0] // 8):
            for j in range(b.shape[1] // 128):
                t = b[8 * i:8 * i + 8, 128 * j:128 * j + 128]
                acc = t if acc is None else acc | t
    return acc & zero


def _after(w, token):
    if token is None:
        return w
    b = pltpu.bitcast(w, u32)
    return pltpu.bitcast(jnp.concatenate([b[0:8] | token, b[8:]], axis=0), bf16)


def _regroup(xs, lane):
    def sel(c, a, b):
        if a is None and b is None:
            return None
        return jnp.where(c, 0.0 if a is None else a, 0.0 if b is None else b)

    for bit in (1, 2):
        c = (lane & (32 * bit)) != 0
        xs = [sel(c, xs[h ^ bit], xs[h]) for h in range(4)]
    return xs


def _kernel(x_hbm, wqkv_hbm, wo_hbm, wr_hbm, wg_hbm, wu_hbm, wd_hbm, out_hbm,
            x_ref, xn_ref, x1_ref, q_ref, k_ref, vt_ref, o_ref,
            wqkv_ref, wo_ref, wg_ref, wu_ref, wd_ref,
            s_ref, m_ref, pv_ref, wcur_ref, cur_ref, shift_ref, var_ref,
            wr_ref, wr_rows, x_sem, w_sem, out_sem):
    nrc = S // RC

    def x_copy(c):
        rows = pl.ds(X_EDGES[c], X_EDGES[c + 1] - X_EDGES[c])
        return pltpu.make_async_copy(x_hbm.at[0, rows], x_ref.at[rows], x_sem.at[c])

    def wqkv_copy(part, lo, hi, sem):
        cols = pl.ds(part * D + lo, hi - lo)
        return pltpu.make_async_copy(
            wqkv_hbm.at[:, cols], wqkv_ref.at[:, cols], w_sem.at[sem])

    head_copies = [wqkv_copy(i, 0, 128, i) for i in range(3)]
    next_copies = [wqkv_copy(i, 128, 256, 3 + i) for i in range(3)]
    rest_copies = [wqkv_copy(i, 256, D, 6 + i) for i in range(3)]
    wr_copy = pltpu.make_async_copy(wr_hbm, wr_ref, w_sem.at[9])
    late_copies = [
        pltpu.make_async_copy(src, dst, w_sem.at[10 + i])
        for i, (src, dst) in enumerate(
            [(wo_hbm, wo_ref), (wg_hbm, wg_ref), (wu_hbm, wu_ref), (wd_hbm, wd_ref)])]

    def out_copy(i, r0, n):
        rows = pl.ds(r0, n)
        return pltpu.make_async_copy(x_ref.at[rows], out_hbm.at[0, rows], out_sem.at[i])

    def load_rows(blk, j, go):
        x = x_ref[pl.ds(pl.multiple_of(blk * 128 + j * 16, 16), 16), :].astype(f32)
        if go is None:
            return x
        first = pltpu.bitcast(x[:, 0:128], u32) | jnp.concatenate([go, go], axis=0)
        return jnp.concatenate([pltpu.bitcast(first, f32), x[:, 128:]], axis=1)

    def ln_stats(blk, j, slot, go=None):
        m, v = _row_moments(*_lane_moments(load_rows(blk, j, go)))
        shift_ref[slot, j * 16:(j + 1) * 16, :] = jnp.broadcast_to(
            _round_bf16(m), (16, 128))
        v = jnp.broadcast_to(v, (16, 128))
        return [v[0:8], v[8:16]]

    def ln_gather(slot, vs):
        lane = lax.broadcasted_iota(jnp.int32, (8, 128), 1)
        bit = 1
        while len(vs) > 1:
            vs = [jnp.where((lane & bit) != 0, vs[i + 1], vs[i])
                  for i in range(0, len(vs), 2)]
            bit *= 2
        var_ref[slot] = vs[0]

    def ln_apply(blk, j, slot, scales, go=None):
        shift = shift_ref[slot, j * 16:(j + 1) * 16, :]
        if go is not None:
            shift = pltpu.bitcast(
                pltpu.bitcast(shift, u32) | jnp.concatenate([go, go], axis=0), f32)
        scale = jnp.concatenate(
            [jnp.broadcast_to(scales[:, i:i + 1], (8, 128)) for i in (2 * j, 2 * j + 1)],
            axis=0)
        ln = (load_rows(blk, j, None) - _widen(shift)) * _widen(scale)
        cur_ref[slot, j * 16:(j + 1) * 16, :] = ln.astype(bf16)

    def stage_weights(g):
        for part in range(3):
            cols = pl.ds(pl.multiple_of(part * D + g * 128, 128), 128)
            wcur_ref[part] = pltpu.bitcast(wqkv_ref[:, cols], u32)

    def project(part, blk, xn):
        y = jnp.dot(pltpu.bitcast(xn, bf16), pltpu.bitcast(wcur_ref[part], bf16),
                    preferred_element_type=f32)
        marks = (y[0:8], y[64:72])
        if part == 0:
            y = y * (SCALE * LOG2E)
        if part == 2:
            y = y.T
        (q_ref, k_ref, vt_ref)[part][blk] = pltpu.bitcast(y.astype(bf16), u32)
        return marks

    def tri():
        return (lax.broadcasted_iota(jnp.int32, (16, 128), 0)
                - (lax.broadcasted_iota(jnp.int32, (16, 128), 1) & 31))

    def scores(t):
        slot = t % 2
        head = lax.broadcasted_iota(jnp.int32, (16, 128), 1) >> 5
        tiles = []
        for j in range(4):
            k0 = t * 128 + j * 32 - 256
            order = [c for c in [0, 16, 1, 17] + list(range(2, 16)) if k0 + 16 * c >= 0]
            parts = []
            for c in order:
                key = k0 + 16 * c
                parts.append(k_ref[key // 128, key % 128 // 2:key % 128 // 2 + 8, :])
            kw = pltpu.bitcast(jnp.concatenate(parts, axis=0), bf16)
            qt = q_ref[t, j * 16:(j + 1) * 16, :]
            w = jnp.concatenate(
                [jnp.where(head == (s ^ j), qt, jnp.zeros_like(qt)) for s in range(4)],
                axis=0)
            sc = lax.dot_general(kw, pltpu.bitcast(w, bf16), (((1,), (1,)), ((), ())),
                                 preferred_element_type=f32)
            tiles.append({c: sc[16 * i:16 * i + 16] for i, c in enumerate(order)})
        d = tri()
        ms = [None] * 4
        for c in range(16):
            for j in range(4):
                if c < 2:
                    sm = jnp.where(d > -16 * c, tiles[j].get(c, NEG), tiles[j][c + 16])
                elif c in tiles[j]:
                    sm = tiles[j][c]
                else:
                    continue
                s_ref[slot, j, 16 * c:16 * c + 16, :] = sm
                mm = jnp.maximum(sm[0:8], sm[8:16])
                ms[j] = mm if ms[j] is None else jnp.maximum(ms[j], mm)
        for j in range(4):
            m_ref[slot, j] = jnp.broadcast_to(
                jnp.max(ms[j], axis=0, keepdims=True), (8, 128))

    def attend(g, t):
        slot = t % 2
        d = tri()
        lane = lax.broadcasted_iota(jnp.int32, (16, 128), 1)
        m2 = [jnp.concatenate([m_ref[slot, j]] * 2, axis=0) for j in range(4)]
        l = [None] * 4
        probs = {}

        def prob(j, key):
            c = (key - (t * 128 + j * 32 - 256)) // 16
            if c < 0 or c >= 18:
                return None
            cm = c % 16
            if (j, cm) not in probs:
                p = jnp.exp2(s_ref[slot, j, 16 * cm:16 * cm + 16, :] - m2[j])
                pp = p[0:8] + p[8:16]
                l[j] = pp if l[j] is None else l[j] + pp
                probs[(j, cm)] = p
            p = probs[(j, cm)]
            if c < 2:
                return jnp.where(d > -16 * cm, p, 0.0)
            if c >= 16:
                return jnp.where(d > -16 * cm, 0.0, p)
            return p

        o = [None] * 4
        for kb in range(t - 2, t + 1):
            if kb > t - 2:
                yield
            if kb < 0:
                continue
            rows = [[None] * 8 for _ in range(4)]
            for c in reversed(range(8)):
                xs = _regroup([prob(j, kb * 128 + c * 16) for j in range(4)], lane)
                for h in range(4):
                    rows[h][c] = xs[h]
            for h in range(4):
                p = jnp.concatenate(rows[h], axis=0).astype(bf16)
                vt = pltpu.bitcast(vt_ref[kb, h * 16:(h + 1) * 16, :], bf16)
                part = jnp.dot(vt, p, preferred_element_type=f32)
                if kb < t:
                    pv_ref[t - 1 - kb, h] = part
                else:
                    for i in range(min(t, 2)):
                        part = part + pv_ref[i, h]
                    o[h] = part
        inv = _regroup(
            [1.0 / jnp.sum(l[j], axis=0, keepdims=True) for j in range(4)], lane[0:1])
        ot = jnp.concatenate([o[h] * inv[h] for h in range(4)], axis=0).T
        out = _regroup([ot[32 * s:32 * s + 32] for s in range(4)],
                       lax.broadcasted_iota(jnp.int32, (32, 128), 1))
        o_ref[g, t] = pltpu.bitcast(jnp.concatenate(out, axis=0).astype(bf16), u32)
        yield

    def layer(li, carry):
        first = li == 0
        izero = li >> 1
        zero = izero.astype(u32)

        @pl.when(first)
        def _():
            x_copy(0).start()
            wr_copy.start()
            for cp in head_copies:
                cp.start()
            x_copy(1).start()
            wr_copy.wait()
            wr_rows[...] = jnp.broadcast_to(
                wr_ref[...].astype(f32).reshape(1, D), (16, D))
            x_copy(0).wait()

        for blk in range(2):
            ln_gather(blk, [v for j in range(8) for v in ln_stats(blk, j, blk)])
        scales = _inv_std(var_ref[0])
        for j in range(8):
            ln_apply(izero, j, 0, scales)

        @pl.when(first)
        def _():
            for cp in head_copies:
                cp.wait()
            x_copy(2).start()

        stage_weights(0)

        def norm_body(c, _):
            for i in range(nrc):
                @pl.when(jnp.logical_and(first, c == i))
                def _():
                    x_copy(i + 1).wait()
                    if i + 3 < len(X_EDGES) - 1:
                        x_copy(i + 3).start()
                    for cp in ([], next_copies, rest_copies, [])[i]:
                        cp.start()

            go = [None, None]
            for b in range(RC // 128):
                blk = c * (RC // 128) + b
                xn = pltpu.bitcast(cur_ref[b % 2], u32)
                xn_ref[pl.ds(pl.multiple_of(blk * 64, 64), 64), :] = xn
                scales = _inv_std(var_ref[(b + 1) % 2])
                vs = []
                for i, part in enumerate((2, 0, 1)):
                    for h in range(2):
                        for j in APPLY_AT[2 * i + h]:
                            ln_apply(jnp.minimum(blk + 1, NT - 1), j, (b + 1) % 2,
                                     scales, go[h])
                        for j in STATS_AT[2 * i + h]:
                            vs += ln_stats(jnp.minimum(blk + 2, NT - 1), j, b % 2, go[h])
                    go = [_token([m], zero) for m in project(part, blk, xn)]
                ln_gather(b % 2, vs)
            return _

        lax.fori_loop(0, nrc, norm_body, None)

        @pl.when(first)
        def _():
            for cp in next_copies:
                cp.wait()

        def att_body(g, _):
            def nxt(part, blk):
                if 0 <= blk < NT:
                    project(part, blk, xn_ref[blk * 64:(blk + 1) * 64, :])

            @pl.when(jnp.logical_and(first, g == 1))
            def _():
                for cp in rest_copies:
                    cp.wait()
                for cp in late_copies:
                    cp.start()

            stage_weights(g + 1)
            scores(0)
            for t in range(NT):
                if t + 1 < NT:
                    scores(t + 1)
                steps = attend(g, t)
                for part in range(3):
                    nxt(part, t - part)
                    next(steps)
            nxt(2, NT - 2)
            nxt(2, NT - 1)
            nxt(1, NT - 1)
            return _

        lax.fori_loop(0, NG - 1, att_body, None)

        @pl.when(first)
        def _():
            for cp in late_copies:
                cp.wait()

        stats = {}
        wr_sum = jnp.sum(wr_rows[...], axis=-1, keepdims=True)
        best = jnp.full((8, 1), -jnp.inf, f32)
        best_i = jnp.zeros((8, 1), jnp.int32)
        sub = lax.broadcasted_iota(jnp.int32, (8, 1), 0)
        toks = [None] * 8
        scores(0)
        for t in range(NT):
            if t + 1 < NT:
                scores(t + 1)
            steps = attend(NG - 1, t)
            o = pltpu.bitcast(jnp.concatenate(
                [o_ref[g, t] for g in range(EARLY)], axis=1), bf16)
            for j in range(4):
                blk = (slice(t * 128, (t + 1) * 128), slice(j * 256, (j + 1) * 256))
                x1_ref[blk] = x_ref[blk].astype(f32) + jnp.dot(
                    o, wo_ref[0:EARLY * 128, blk[1]], preferred_element_type=f32)
                if j < 3:
                    next(steps)
        for t in range(NT + 1):
            for j in range(8):
                if t < NT:
                    o = pltpu.bitcast(jnp.concatenate(
                        [o_ref[g, t] for g in range(EARLY, NG)], axis=1), bf16)
                    w = _after(wo_ref[EARLY * 128:, j * 128:(j + 1) * 128], toks[-6])
                    a = jnp.dot(o, w, preferred_element_type=f32)
                    blk = (slice(t * 128, (t + 1) * 128), slice(j * 128, (j + 1) * 128))
                    x1_ref[blk] = a + x1_ref[blk]
                    go = _token([a[0:8]], zero)
                done = []
                p = (t - 1) * 8 + j
                if t > 0:
                    x1 = x1_ref[p * 16:(p + 1) * 16, :]
                    if t < NT:
                        x1 = pltpu.bitcast(pltpu.bitcast(x1, u32) | _widen(
                            jnp.concatenate([go, go], axis=0)), f32)
                    moments = _lane_moments(x1)
                    shift, scale = _row_stats(*moments)
                    xw = jnp.sum(x1 * wr_rows[...], axis=-1, keepdims=True)
                    stats[p] = (1.0 + scale, shift * scale, (xw - shift * wr_sum) * scale)
                    done += moments
                last = p == S // 16 - 1
                for f in range(max(p - LAG, 0), p + 1 if last else p - LAG + 1):
                    r0 = f * 16
                    gain, offset, r = stats[f]
                    rows = pl.ds(pl.multiple_of(izero * 16 + r0, 16), 16)
                    x2 = (x1_ref[rows, :] * gain - offset).astype(bf16)
                    x_ref[r0:r0 + 16, :] = x2
                    for i in range(2):
                        ri = r[8 * i:8 * i + 8]
                        take = ri > best
                        best = jnp.where(take, ri, best)
                        best_i = jnp.where(take, sub + (r0 + 8 * i), best_i)
                    done += [jnp.broadcast_to(best, (8, 128))]
                    if (r0 + 16) % OUT_ROWS == 0:
                        out_copy(r0 // OUT_ROWS, r0 + 16 - OUT_ROWS, OUT_ROWS).start()
                toks.append(_token(done, zero) if done else None)

        top = jnp.max(best, axis=0, keepdims=True)
        idx = jnp.min(jnp.where(best == top, best_i, S - 1))
        base = pl.multiple_of((idx >> 4) << 4, 16)
        tile = pl.ds(base, 16)
        x1 = x1_ref[tile, :]
        shift, scale = _row_stats(*_lane_moments(x1))
        ln = (x1 - shift) * scale
        xs = ln.astype(bf16)
        gate = jnp.dot(xs, wg_ref[...], preferred_element_type=f32)
        up = jnp.dot(xs, wu_ref[...], preferred_element_type=f32)
        hid = (gate * jax.nn.sigmoid(gate) * up).astype(bf16)
        y = None
        weight = jax.nn.sigmoid(top)
        for j in range(F // 512):
            part = jnp.dot(hid[:, j * 512:(j + 1) * 512], wd_ref[j * 512:(j + 1) * 512, :],
                           preferred_element_type=f32) * weight
            y = part if y is None else y + part
        xt = x_ref[tile, :].astype(f32)
        hit = lax.broadcasted_iota(jnp.int32, (16, D), 0) == idx - base
        new = jnp.where(hit, x1 + ln + y, xt).astype(bf16)
        for i in range(S // OUT_ROWS):
            out_copy(i, i * OUT_ROWS, OUT_ROWS).wait()
        x_ref[tile, :] = new

        @pl.when(jnp.logical_not(first))
        def _():
            fix = out_copy(0, base, 16)
            fix.start()
            fix.wait()

        return carry

    lax.fori_loop(0, 2, layer, None)


@jax.jit
def pallas_interleave_layers__sliding_block__moe_arch_mod__prompt_kernel(
    A_x: jax.Array,
    A_wqkv: jax.Array,
    A_wo: jax.Array,
    B_x: jax.Array,
    B_w_r: jax.Array,
    B_w_gate: jax.Array,
    B_w_up: jax.Array,
    B_w_down: jax.Array,
):
    del B_x
    hbm = pl.BlockSpec(memory_space=pl.ANY)
    return pl.pallas_call(
        _kernel,
        out_shape=jax.ShapeDtypeStruct((1, S, D), bf16),
        in_specs=[hbm] * 7,
        out_specs=hbm,
        scratch_shapes=[
            pltpu.VMEM((S, D), bf16),
            pltpu.VMEM((S // 2, D), u32),
            pltpu.VMEM((S, D), f32),
            pltpu.VMEM((NT, 64, 128), u32),
            pltpu.VMEM((NT, 64, 128), u32),
            pltpu.VMEM((NT, 64, 128), u32),
            pltpu.VMEM((NG, NT, 64, 128), u32),
            pltpu.VMEM((D, 3 * D), bf16),
            pltpu.VMEM((D, D), bf16),
            pltpu.VMEM((D, F), bf16),
            pltpu.VMEM((D, F), bf16),
            pltpu.VMEM((F, D), bf16),
            pltpu.VMEM((2, 4, 256, 128), f32),
            pltpu.VMEM((2, 4, 8, 128), f32),
            pltpu.VMEM((2, 4, 32, 128), f32),
            pltpu.VMEM((3, D // 2, 128), u32),
            pltpu.VMEM((2, 128, D), bf16),
            pltpu.VMEM((2, 128, 128), f32),
            pltpu.VMEM((2, 8, 128), f32),
            pltpu.VMEM((D,), bf16),
            pltpu.VMEM((16, D), f32),
            pltpu.SemaphoreType.DMA((len(X_EDGES) - 1,)),
            pltpu.SemaphoreType.DMA((14,)),
            pltpu.SemaphoreType.DMA((S // OUT_ROWS,)),
        ],
        compiler_params=pltpu.CompilerParams(vmem_limit_bytes=100 * 2**20),
    )(A_x, A_wqkv, A_wo, B_w_r, B_w_gate, B_w_up, B_w_down)
```
